```python
import jax
import jax.numpy as jnp

def _softmax(x, axis=-1):
    return jax.nn.softmax(x, axis=axis)
def _gelu(x):
    return jax.nn.gelu(x, approximate=True)
def _silu(x):
    return jax.nn.silu(x)
def _sigmoid(x):
    return jax.nn.sigmoid(x)
def _layernorm(x, axis=-1, eps=1e-5):
    m = jnp.mean(x, axis=axis, keepdims=True)
    v = jnp.var(x, axis=axis, keepdims=True)
    return (x - m) / jnp.sqrt(v + eps)
def _scatter_add(tgt, idx, src, axis=0):
    return tgt.at[idx].add(src)
def _segment_sum(src, seg, n):
    return jax.ops.segment_sum(src, seg, n)
class _Rng:
    def __init__(self, key):
        self._k = key
    def _next(self):
        self._k, sub = jax.random.split(self._k)
        return sub
    def normal(self, shape):
        return jax.random.normal(self._next(), shape, dtype=jnp.bfloat16)
    def randint(self, lo, hi, shape):
        return jax.random.randint(self._next(), shape, lo, hi, dtype=jnp.int32)
    def uniform(self, shape, lo=0.0, hi=1.0):
        return jax.random.uniform(self._next(), shape, jnp.bfloat16, lo, hi)
    def permutation(self, n):
        return jax.random.permutation(self._next(), n)


kernel_name = 'sequential_preLN__sliding_block__glu_gated_glu__prompt'

def _fwd_setup_inputs():
    _rng = _Rng(jax.random.key(int.from_bytes(__import__("os").urandom(4), "little")))
    _w = (lambda a: (lambda t: t.astype(jnp.bfloat16) if jnp.issubdtype(t.dtype, jnp.floating) else t)(jnp.asarray(a)))
    def _A_setup():
        B, S, D = 1, 2048, 512
        return {
            "x": _w((lambda *s: _rng.normal(s) * 0.05)(B, S, D)),
            "wqkv": _w((lambda *s: _rng.normal(s) * 0.05)(D, 3 * D)),
            "wo": _w((lambda *s: _rng.normal(s) * 0.05)(D, D)),
        }
    _A_in = _A_setup()

    def _B_setup():
        B, S, D, F = 1, 2048, 512, 1376
        return {
            "x": _w((lambda *s: _rng.normal(s) * 0.05)(B, S, D)),
            "w_gate": _w((lambda *s: _rng.normal(s) * 0.05)(D, F)),
            "w_up": _w((lambda *s: _rng.normal(s) * 0.05)(D, F)),
            "w_down": _w((lambda *s: _rng.normal(s) * 0.05)(F, D)),
        }
    _B_in = _B_setup()

    return {
        "A_x": _A_in["x"],
        "A_wqkv": _A_in["wqkv"],
        "A_wo": _A_in["wo"],
        "B_x": _B_in["x"],
        "B_w_gate": _B_in["w_gate"],
        "B_w_up": _B_in["w_up"],
        "B_w_down": _B_in["w_down"],
    }

def _fwd_reference(A_x, A_wqkv, A_wo, B_x, B_w_gate, B_w_up, B_w_down):
    def _A_ref(x, wqkv, wo):
        B, S, D = x.shape
        H = 32; Dh = D // H; W = 256
        qkv = (lambda x, *d: x.transpose(*d))((x @ wqkv).reshape(B, S, 3, H, Dh), 2, 0, 3, 1, 4)
        q, k, v = qkv[0], qkv[1], qkv[2]
        scores = jnp.einsum("bhqd,bhkd->bhqk", q, k) * (Dh ** -0.5)
        idx = jnp.arange(S)
        mask = (idx[:, None] - idx[None, :] >= 0) & (idx[:, None] - idx[None, :] < W)
        scores = jnp.where(mask[None, None], scores, -1e9)
        p = _softmax(scores, axis=-1)
        o = jnp.einsum("bhqk,bhkd->bhqd", p, v)
        return (lambda x, *d: x.transpose(*d))(o, 0, 2, 1, 3).reshape(B, S, D) @ wo

    def _B_ref(x, w_gate, w_up, w_down):
        g = jnp.einsum("bsd,df->bsf", x, w_gate)
        u = jnp.einsum("bsd,df->bsf", x, w_up)
        h = _sigmoid(g) * u
        return jnp.einsum("bsf,fd->bsd", h, w_down)

    x = A_x
    h = x + _A_ref(_layernorm(x, axis=-1), A_wqkv, A_wo)
    h2 = h + _B_ref(_layernorm(h, axis=-1), B_w_gate, B_w_up, B_w_down)
    return h2


def setup_inputs():
    _inp = _fwd_setup_inputs()
    _gk = jax.random.fold_in(jax.random.key(int.from_bytes(__import__("os").urandom(4), "little")), 2**31 - 1)
    _shapes = [[1, 2048, 512]]
    _dtypes = ['bfloat16']
    _gks = jax.random.split(_gk, len(_shapes))
    _gs = [jax.random.normal(k, s, dtype=jnp.dtype(d)) * 0.05 for k, s, d in zip(_gks, _shapes, _dtypes)]
    _inp["grad_out"] = _gs[0]
    return _inp

def reference(A_x, A_wqkv, A_wo, B_w_gate, B_w_up, B_w_down, B_x, grad_out):
    _const = dict(B_x=B_x)
    def _f(*_d):
        return _fwd_reference(**{'A_x': _d[0], 'A_wqkv': _d[1], 'A_wo': _d[2], 'B_w_gate': _d[3], 'B_w_up': _d[4], 'B_w_down': _d[5], **_const})
    _out, _vjp = jax.vjp(_f, A_x, A_wqkv, A_wo, B_w_gate, B_w_up, B_w_down)
    _grads = _vjp(grad_out)
    _out0 = jnp.asarray(_out)
    return (_out0, *[jnp.asarray(_g) for _g in _grads])
```

```python
import jax
import jax.numpy as jnp
from jax import lax
import jax.experimental.pallas as pl
import jax.experimental.pallas.tpu as pltpu

S, D, F = 2048, 512, 1376
H, DH = 32, 16
T = 128
NT = S // T
G = D // 128
RB = 256
NRB = S // RB
TPB = RB // T
EPS = 1e-5
LOG2E = 1.4426950408889634
QSCALE = 0.25 * LOG2E
BF = jnp.bfloat16
F32 = jnp.float32


def _nn(a, b):
    return jnp.dot(a, b, preferred_element_type=F32)


def _nt(a, b):
    return lax.dot_general(a, b, (((1,), (1,)), ((), ())), preferred_element_type=F32)


def _ln(x):
    m = jnp.mean(x, axis=-1, keepdims=True)
    xc = x - m
    v = jnp.mean(xc * xc, axis=-1, keepdims=True)
    r = lax.rsqrt(v + EPS)
    return xc * r, r


def _ln_bwd(dy, xn, r):
    a = jnp.mean(dy, axis=-1, keepdims=True)
    b = jnp.mean(dy * xn, axis=-1, keepdims=True)
    return r * (dy - a - xn * b)


def _kernel(x_hbm, wqkv_hbm, wo_hbm, wg_hbm, wu_hbm, wd_hbm, do_hbm,
            out_hbm, dx_hbm, dwqkv_hbm, dwo_hbm, dwg_hbm, dwu_hbm, dwd_hbm,
            x_v, wqkv_v, wo_v, wg_v, wu_v, wd_v, dout_v,
            xn1t, kn, vn, qt, kt, vt, ot, linv, p_s, h_s, dot_s, delta, dqt, dkt, dvt,
            acc_g, acc_u, acc_d, acc_o, acc_qkv,
            out_v, dx_v, og_v, ou_v, od_v, oo_v, oqkv_v, sems):
    def cp(src, dst, i):
        return pltpu.make_async_copy(src, dst, sems.at[i])

    in_cps = [cp(x_hbm, x_v, 0), cp(wqkv_hbm, wqkv_v, 1), cp(wo_hbm, wo_v, 2), cp(do_hbm, dout_v, 3),
              cp(wg_hbm, wg_v, 4), cp(wu_hbm, wu_v, 5), cp(wd_hbm, wd_v, 6)]
    for c in in_cps[:2]:
        c.start()
    in_cps[0].wait()
    in_cps[1].wait()
    for c in in_cps[2:]:
        c.start()

    def phase_a(b, c):
        rows = pl.ds(pl.multiple_of(b * RB, RB), RB)
        xn, _ = _ln(x_v[rows, :].astype(F32))
        qkv = _nn(xn.astype(BF), wqkv_v[...])
        q = qkv[:, :D] * QSCALE
        k = qkv[:, D:2 * D]
        v = qkv[:, 2 * D:]
        for g in range(G):
            kn[g, rows, :] = k[:, g * 128:(g + 1) * 128].astype(BF)
            vn[g, rows, :] = v[:, g * 128:(g + 1) * 128].astype(BF)
        for t in range(TPB):
            r = slice(t * T, (t + 1) * T)
            j = b * TPB + t
            xn1t[b, :, r] = xn[r].T.astype(BF)
            qt[j] = q[r].T.astype(BF)
            kt[j] = k[r].T.astype(BF)
            vt[j] = v[r].T.astype(BF)
        return c
    lax.fori_loop(0, NRB, phase_a, 0)

    kk = lax.broadcasted_iota(jnp.int32, (T, T), 0)
    qq = lax.broadcasted_iota(jnp.int32, (T, T), 1)
    hrow = lax.broadcasted_iota(jnp.int32, (T, T), 0) // DH

    def attn_fwd(i, g, nt):
        grow = pl.ds(pl.multiple_of(g * 128, 128), 128)
        qg = qt[i, grow, :]
        k0 = pl.multiple_of((i - (nt - 1)) * T, T)
        keys = kn[g, pl.ds(k0, nt * T), :]
        for h in range(8):
            hr = pl.ds(pl.multiple_of(g * 128 + h * DH, DH), DH)
            s = _nn(keys, jnp.where(hrow == h, qg, jnp.zeros_like(qg)))
            sd = s[(nt - 1) * T:]
            if nt == 3:
                sm = jnp.where(kk > qq, s[:T], sd)
            else:
                sm = jnp.where(kk > qq, -1e9, sd)
            mx = jnp.max(sm, axis=0, keepdims=True)
            if nt > 1:
                s1 = s[(nt - 2) * T:(nt - 1) * T]
                mx = jnp.maximum(mx, jnp.max(s1, axis=0, keepdims=True))
                p1 = jnp.exp2(s1 - mx)
            pm = jnp.exp2(sm - mx)
            l = jnp.sum(pm, axis=0, keepdims=True)
            zero = jnp.zeros_like(pm)
            acc = _nn(vt[i, hr, :], jnp.where(kk > qq, zero, pm).astype(BF))
            p_s[i, g * 8 + h, 0] = pm.astype(BF)
            if nt > 1:
                l = l + jnp.sum(p1, axis=0, keepdims=True)
                p1b = p1.astype(BF)
                p_s[i, g * 8 + h, 1] = p1b
                acc = acc + _nn(vt[i - 1, hr, :], p1b)
            if nt > 2:
                acc = acc + _nn(vt[i - 2, hr, :], jnp.where(kk > qq, pm, zero).astype(BF))
            li = 1.0 / l
            linv[i, g, h:h + 1, :] = li
            ot[i, hr, :] = (acc * li).astype(BF)

    def run_attn(fn):
        lax.fori_loop(0, G, lambda g, c: (fn(0, g, 1), c)[1], 0)
        lax.fori_loop(0, G, lambda g, c: (fn(1, g, 2), c)[1], 0)
        lax.fori_loop(0, (NT - 2) * G, lambda n, c: (fn(2 + n // G, n % G, 3), c)[1], 0)

    run_attn(attn_fwd)

    for c in in_cps[2:]:
        c.wait()
    acc_g[...] = jnp.zeros_like(acc_g)
    acc_u[...] = jnp.zeros_like(acc_u)
    acc_d[...] = jnp.zeros_like(acc_d)
    acc_o[...] = jnp.zeros_like(acc_o)

    def phase_c(b, c):
        rows = pl.ds(pl.multiple_of(b * RB, RB), RB)
        otb = jnp.concatenate([ot[b * TPB + t] for t in range(TPB)], axis=1)
        o = otb.astype(F32).T.astype(BF)
        h = x_v[rows, :].astype(F32) + _nn(o, wo_v[...])
        xn, r = _ln(h)
        xnb = xn.astype(BF)
        g = _nn(xnb, wg_v[...])
        u = _nn(xnb, wu_v[...])
        sg = jax.nn.sigmoid(g)
        hh = (sg * u).astype(BF)
        out_v[rows, :] = (h + _nn(hh, wd_v[...])).astype(BF)
        dout = dout_v[rows, :]
        doutf = dout.astype(F32)
        acc_d[...] += _nn(doutf.T.astype(BF), hh)
        dhh = _nt(dout, wd_v[...])
        du = dhh * sg
        dg = (du * u * (1.0 - sg)).astype(BF)
        du = du.astype(BF)
        xnt = xn.T.astype(BF)
        acc_g[...] += _nn(xnt, dg)
        acc_u[...] += _nn(xnt, du)
        dxn = _nt(dg, wg_v[...]) + _nt(du, wu_v[...])
        dh = doutf + _ln_bwd(dxn, xn, r)
        h_s[rows, :] = dh
        dhb = dh.astype(BF)
        acc_o[...] += _nn(otb, dhb)
        do = _nt(dhb, wo_v[...])
        for t in range(TPB):
            j = b * TPB + t
            dt = do[t * T:(t + 1) * T].T
            for g_ in range(G):
                for h_ in range(8):
                    hr = slice(g_ * 128 + h_ * DH, g_ * 128 + (h_ + 1) * DH)
                    d = dt[hr] * linv[j, g_, h_:h_ + 1, :]
                    dot_s[j, hr, :] = d.astype(BF)
                    delta[j, g_, h_:h_ + 1, :] = jnp.sum(
                        d * otb[hr, t * T:(t + 1) * T].astype(F32), axis=0, keepdims=True)
        return c
    lax.fori_loop(0, NRB, phase_c, 0)

    og_v[...] = acc_g[...].astype(BF)
    ou_v[...] = acc_u[...].astype(BF)
    od_v[...] = acc_d[...].T.astype(BF)
    oo_v[...] = acc_o[...].astype(BF)
    out_cps = [cp(out_v, out_hbm, 7), cp(og_v, dwg_hbm, 8), cp(ou_v, dwu_hbm, 9),
               cp(od_v, dwd_hbm, 10), cp(oo_v, dwo_hbm, 11)]
    for c in out_cps:
        c.start()

    dkt[...] = jnp.zeros_like(dkt)
    dvt[...] = jnp.zeros_like(dvt)

    def attn_bwd(i, g, nt):
        grow = pl.ds(pl.multiple_of(g * 128, 128), 128)
        dg_ = dot_s[i, grow, :]
        k0 = pl.multiple_of((i - (nt - 1)) * T, T)
        vals = vn[g, pl.ds(k0, nt * T), :]
        for h in range(8):
            hr = pl.ds(pl.multiple_of(g * 128 + h * DH, DH), DH)
            dp = _nn(vals, jnp.where(hrow == h, dg_, jnp.zeros_like(dg_)))
            dl = delta[i, g, h:h + 1, :]
            do_h = dot_s[i, hr, :]
            q_h = qt[i, hr, :]
            pmb = p_s[i, g * 8 + h, 0]
            pm = pmb.astype(F32)
            dd = dp[(nt - 1) * T:]
            if nt == 3:
                dd = jnp.where(kk > qq, dp[:T], dd)
            dsm = pm * (dd - dl)
            zero = jnp.zeros_like(pm)

            def tile(j, pb, dsb):
                dvt[j, hr, :] += _nt(do_h, pb)
                dkt[j, hr, :] += _nt(q_h, dsb)
                return _nn(kt[j, hr, :], dsb)

            if nt == 3:
                dq = tile(i, jnp.where(kk > qq, zero, pm).astype(BF), jnp.where(kk > qq, zero, dsm).astype(BF))
                dq += tile(i - 2, jnp.where(kk > qq, pm, zero).astype(BF), jnp.where(kk > qq, dsm, zero).astype(BF))
            else:
                dq = tile(i, pmb, dsm.astype(BF))
            if nt > 1:
                p1b = p_s[i, g * 8 + h, 1]
                ds1 = p1b.astype(F32) * (dp[(nt - 2) * T:(nt - 1) * T] - dl)
                dq += tile(i - 1, p1b, ds1.astype(BF))
            dqt[i, hr, :] = (dq * 0.25).astype(BF)

    run_attn(attn_bwd)

    acc_qkv[...] = jnp.zeros_like(acc_qkv)

    def phase_e(b, c):
        rows = pl.ds(pl.multiple_of(b * RB, RB), RB)
        cat = lambda ref: jnp.concatenate([ref[b * TPB + t] for t in range(TPB)], axis=1)
        dqkv = jnp.concatenate([cat(dqt), (cat(dkt) * (1.0 / LOG2E)).astype(BF), cat(dvt).astype(BF)], axis=0)
        acc_qkv[...] += _nt(xn1t[b], dqkv)
        dxn = _nn(wqkv_v[...], dqkv).T
        xn, r = _ln(x_v[rows, :].astype(F32))
        dx_v[rows, :] = (h_s[rows, :] + _ln_bwd(dxn, xn, r)).astype(BF)
        return c
    lax.fori_loop(0, NRB, phase_e, 0)

    c1 = cp(dx_v, dx_hbm, 12)
    c1.start()
    oqkv_v[...] = acc_qkv[...].astype(BF)
    c2 = cp(oqkv_v, dwqkv_hbm, 13)
    c2.start()
    for c in out_cps + [c1, c2]:
        c.wait()


@jax.jit
def pallas_sequential_preLN__sliding_block__glu_gated_glu__prompt_kernel(
    A_x: jax.Array,
    A_wqkv: jax.Array,
    A_wo: jax.Array,
    B_x: jax.Array,
    B_w_gate: jax.Array,
    B_w_up: jax.Array,
    B_w_down: jax.Array,
    grad_out: jax.Array,
):
    del B_x
    V = pltpu.VMEM
    tb = lambda dt: V((NT, D, T), dt)
    scratch = [
        V((S, D), BF), V((D, 3 * D), BF), V((D, D), BF), V((D, F), BF), V((D, F), BF), V((F, D), BF), V((S, D), BF),
        V((NRB, D, RB), BF), V((G, S, 128), BF), V((G, S, 128), BF), tb(BF), tb(BF), tb(BF), tb(BF),
        V((NT, G, 8, T), F32), V((NT, H, 2, T, T), BF), V((S, D), F32), tb(BF), V((NT, G, 8, T), F32),
        tb(BF), tb(F32), tb(F32),
        V((D, F), F32), V((D, F), F32), V((D, F), F32), V((D, D), F32), V((D, 3 * D), F32),
        V((S, D), BF), V((S, D), BF), V((D, F), BF), V((D, F), BF), V((F, D), BF), V((D, D), BF), V((D, 3 * D), BF),
        pltpu.SemaphoreType.DMA((14,)),
    ]
    sd = jax.ShapeDtypeStruct
    outs = pl.pallas_call(
        _kernel,
        out_shape=(sd((S, D), BF), sd((S, D), BF), sd((D, 3 * D), BF), sd((D, D), BF),
                   sd((D, F), BF), sd((D, F), BF), sd((F, D), BF)),
        in_specs=[pl.BlockSpec(memory_space=pl.ANY)] * 7,
        out_specs=[pl.BlockSpec(memory_space=pl.ANY)] * 7,
        scratch_shapes=scratch,
        compiler_params=pltpu.CompilerParams(vmem_limit_bytes=127 * 1024 * 1024),
    )(A_x.reshape(S, D), A_wqkv, A_wo, B_w_gate, B_w_up, B_w_down, grad_out.reshape(S, D))
    return (outs[0].reshape(1, S, D), outs[1].reshape(1, S, D)) + tuple(outs[2:])
```

```python
import jax
import jax.numpy as jnp
from jax import lax
import jax.experimental.pallas as pl
import jax.experimental.pallas.tpu as pltpu

S, D, F = 2048, 512, 1376
H, DH = 32, 16
T = 128
NT = S // T
G = D // 128
RB = 256
NRB = S // RB
TPB = RB // T
GP = 4
LA = 10
EPS = 1e-5
LOG2E = 1.4426950408889634
QSCALE = 0.25 * LOG2E
BF = jnp.bfloat16
F32 = jnp.float32


def _nn(a, b):
    return jnp.dot(a, b, preferred_element_type=F32)


def _nt(a, b):
    return lax.dot_general(a, b, (((1,), (1,)), ((), ())), preferred_element_type=F32)


def _ln(x):
    m = jnp.mean(x, axis=-1, keepdims=True)
    xc = x - m
    v = jnp.mean(xc * xc, axis=-1, keepdims=True)
    r = lax.rsqrt(v + EPS)
    return xc * r, r


def _ln_bwd(dy, xn, r):
    a = jnp.mean(dy, axis=-1, keepdims=True)
    b = jnp.mean(dy * xn, axis=-1, keepdims=True)
    return r * (dy - a - xn * b)


def _kernel(x_hbm, wqkv_hbm, wo_hbm, wg_hbm, wu_hbm, wd_hbm, do_hbm,
            out_hbm, dx_hbm, dwqkv_hbm, dwo_hbm, dwg_hbm, dwu_hbm, dwd_hbm,
            x_v, wqkv_v, wo_v, wg_v, wu_v, wd_v, dout_v,
            xn1t, kn, vn, qt, kt, vt, ot, linv, p_s, h_s, dot_s, delta, dqt, dkt, dvt,
            acc_g, acc_u, acc_d, acc_o, acc_qkv,
            out_v, dx_v, og_v, ou_v, od_v, oo_v, oqkv_v, sems):
    def cp(src, dst, i):
        return pltpu.make_async_copy(src, dst, sems.at[i])

    x_cps = [cp(x_hbm.at[:RB], x_v.at[:RB], 0), cp(x_hbm.at[RB:], x_v.at[RB:], 14)]
    w_cp = cp(wqkv_hbm, wqkv_v, 1)
    in_cps = [None, None, cp(wo_hbm, wo_v, 2), cp(do_hbm, dout_v, 3),
              cp(wg_hbm, wg_v, 4), cp(wu_hbm, wu_v, 5), cp(wd_hbm, wd_v, 6)]
    x_cps[0].start()
    w_cp.start()
    x_cps[1].start()
    for ref in (acc_g, acc_u, acc_d, acc_o, acc_qkv, dkt, dvt):
        ref[...] = jnp.zeros_like(ref)
    x_cps[0].wait()
    w_cp.wait()
    x_cps[1].wait()
    for c in in_cps[2:]:
        c.start()

    def phase_a(b, c):
        rows = pl.ds(pl.multiple_of(b * RB, RB), RB)
        xn, _ = _ln(x_v[rows, :].astype(F32))
        qkv = _nn(xn.astype(BF), wqkv_v[...])
        q = qkv[:, :D] * QSCALE
        k = qkv[:, D:2 * D]
        v = qkv[:, 2 * D:]
        for g in range(G):
            kn[g, rows, :] = k[:, g * 128:(g + 1) * 128].astype(BF)
            vn[g, rows, :] = v[:, g * 128:(g + 1) * 128].astype(BF)
        for t in range(TPB):
            r = slice(t * T, (t + 1) * T)
            j = b * TPB + t
            xn1t[b, :, r] = xn[r].T.astype(BF)
            qt[j] = q[r].T.astype(BF)
            kt[j] = k[r].T.astype(BF)
            vt[j] = v[r].T.astype(BF)
        return c
    with jax.named_scope("phA"):
        lax.fori_loop(0, NRB, phase_a, 0)

    kk = lax.broadcasted_iota(jnp.int32, (T, T), 0)
    qq = lax.broadcasted_iota(jnp.int32, (T, T), 1)
    r2 = 2 * lax.broadcasted_iota(jnp.int32, (T // 2, T), 0)
    q2 = lax.broadcasted_iota(jnp.int32, (T // 2, T), 1)
    upper = jnp.where(r2 > q2, 0xFFFF, 0) | jnp.where(r2 + 1 > q2, -0x10000, 0)

    def split(pb):
        w = pltpu.bitcast(pb, jnp.int32)
        old = w & upper
        return pltpu.bitcast(old, BF), pltpu.bitcast(w ^ old, BF)

    def head_w(ref_rows, h):
        parts = [jnp.zeros((h * DH, T), BF)] * (h > 0) + [ref_rows] + [jnp.zeros((T - (h + 1) * DH, T), BF)] * (h < 7)
        return jnp.concatenate(parts, axis=0)

    def attn_fwd(i, g, nt):
        grow = pl.ds(pl.multiple_of(g * 128, 128), 128)
        k0 = pl.multiple_of((i - (nt - 1)) * T, T)
        keys = [kn[g * GP + a, pl.ds(k0, nt * T), :] for a in range(GP)]
        hrs = [pl.ds(pl.multiple_of(g * 128 * GP + h * DH, DH), DH) for h in range(8 * GP)]
        sc = lambda h: _nn(keys[h // 8], head_w(qt[i, hrs[h], :], h % 8))
        q_ = [sc(h) for h in range(LA)]
        for h in range(8 * GP):
            hr = hrs[h]
            s = q_[h]
            if h + LA < 8 * GP:
                q_.append(sc(h + LA))
            sd = s[(nt - 1) * T:]
            if nt == 3:
                sm = jnp.where(kk > qq, s[:T], sd)
            else:
                sm = jnp.where(kk > qq, -1e9, sd)
            mx = jnp.max(sm, axis=0, keepdims=True)
            if nt > 1:
                s1 = s[(nt - 2) * T:(nt - 1) * T]
                mx = jnp.maximum(mx, jnp.max(s1, axis=0, keepdims=True))
                p1 = jnp.exp2(s1 - mx)
            pm = jnp.exp2(sm - mx)
            l = jnp.sum(pm, axis=0, keepdims=True)
            pmb = pm.astype(BF)
            if nt == 3:
                pold, pnew = split(pmb)
            else:
                pnew = pmb
            acc = _nn(vt[i, hr, :], pnew)
            p_s[i, g * 8 * GP + h, 0] = pmb
            if nt > 1:
                l = l + jnp.sum(p1, axis=0, keepdims=True)
                p1b = p1.astype(BF)
                p_s[i, g * 8 * GP + h, 1] = p1b
                acc = acc + _nn(vt[i - 1, hr, :], p1b)
            if nt > 2:
                acc = acc + _nn(vt[i - 2, hr, :], pold)
            li = 1.0 / l
            linv[i, g * GP + h // 8, h % 8:h % 8 + 1, :] = li
            ot[i, hr, :] = (acc * li).astype(BF)

    def run_attn(fn):
        fn(0, 0, 1)
        if fn.__name__ == 'attn_bwd':
            for c in out_cps:
                c.start()
        lax.fori_loop(0, G // GP, lambda g, c: (fn(1, g, 2), c)[1], 0)
        lax.fori_loop(0, (NT - 2) * (G // GP), lambda n, c: (fn(2 + n // (G // GP), n % (G // GP), 3), c)[1], 0)

    with jax.named_scope("phB"):
        run_attn(attn_fwd)

    for c in in_cps[2:]:
        c.wait()

    def phase_c(b, c):
        rows = pl.ds(pl.multiple_of(b * RB, RB), RB)
        otb = jnp.concatenate([ot[b * TPB + t] for t in range(TPB)], axis=1)
        o = otb.astype(F32).T.astype(BF)
        h = x_v[rows, :].astype(F32) + _nn(o, wo_v[...])
        dout = dout_v[rows, :]
        dhh = _nt(dout, wd_v[...])
        xn, r = _ln(h)
        xnb = xn.astype(BF)
        g = _nt(xnb, wg_v[...])
        u = _nt(xnb, wu_v[...])
        sg = 0.5 * jnp.tanh(0.5 * g) + 0.5
        hh = (sg * u).astype(BF)
        out_v[rows, :] = (h + _nn(hh, wd_v[...])).astype(BF)
        doutf = dout.astype(F32)
        du = dhh * sg
        dg = (du * u * (1.0 - sg)).astype(BF)
        du = du.astype(BF)
        xnt = xn.T.astype(BF)
        dxn = _nn(dg, wg_v[...]) + _nn(du, wu_v[...])
        acc_g[...] += _nn(xnt, dg)
        dh = doutf + _ln_bwd(dxn, xn, r)
        h_s[rows, :] = dh
        dhb = dh.astype(BF)
        do = _nt(dhb, wo_v[...])
        acc_u[...] += _nn(xnt, du)
        acc_d[...] += _nn(doutf.T.astype(BF), hh)
        acc_o[...] += _nn(otb, dhb)
        for t in range(TPB):
            j = b * TPB + t
            dt = do[t * T:(t + 1) * T].T
            for g_ in range(G):
                for h_ in range(8):
                    hr = slice(g_ * 128 + h_ * DH, g_ * 128 + (h_ + 1) * DH)
                    d = dt[hr] * linv[j, g_, h_:h_ + 1, :]
                    dot_s[j, hr, :] = d.astype(BF)
                    delta[j, g_, h_:h_ + 1, :] = jnp.sum(
                        d * otb[hr, t * T:(t + 1) * T].astype(F32), axis=0, keepdims=True)
        return c
    with jax.named_scope("phC"):
        lax.fori_loop(0, NRB, phase_c, 0)

    out_cps = [cp(out_v, out_hbm, 7), cp(og_v, dwg_hbm, 8), cp(ou_v, dwu_hbm, 9),
               cp(od_v, dwd_hbm, 10), cp(oo_v, dwo_hbm, 11)]


    def attn_bwd(i, g, nt):
        grow = pl.ds(pl.multiple_of(g * 128, 128), 128)
        k0 = pl.multiple_of((i - (nt - 1)) * T, T)
        vals = [vn[g * GP + a, pl.ds(k0, nt * T), :] for a in range(GP)]
        hrs = [pl.ds(pl.multiple_of(g * 128 * GP + h * DH, DH), DH) for h in range(8 * GP)]
        sc = lambda h: _nn(vals[h // 8], head_w(dot_s[i, hrs[h], :], h % 8))
        q_ = [sc(h) for h in range(LA)]
        for h in range(8 * GP):
            hr = hrs[h]
            dp = q_[h]
            if h + LA < 8 * GP:
                q_.append(sc(h + LA))
            dl = delta[i, g * GP + h // 8, h % 8:h % 8 + 1, :]
            do_h = dot_s[i, hr, :]
            q_h = qt[i, hr, :]
            pmb = p_s[i, g * 8 * GP + h, 0]
            pm = pmb.astype(F32)
            dd = dp[(nt - 1) * T:]
            if nt == 3:
                dd = jnp.where(kk > qq, dp[:T], dd)
            dsm = pm * (dd - dl)

            def tile(j, pb, dsb):
                dvt[j, hr, :] += _nt(do_h, pb)
                dkt[j, hr, :] += _nt(q_h, dsb)
                return _nn(kt[j, hr, :], dsb)

            if nt == 3:
                pold, pnew = split(pmb)
                dold, dnew = split(dsm.astype(BF))
                dq = tile(i, pnew, dnew) + tile(i - 2, pold, dold)
            else:
                dq = tile(i, pmb, dsm.astype(BF))
            if nt > 1:
                p1b = p_s[i, g * 8 * GP + h, 1]
                ds1 = p1b.astype(F32) * (dp[(nt - 2) * T:(nt - 1) * T] - dl)
                dq += tile(i - 1, p1b, ds1.astype(BF))
            dqt[i, hr, :] = (dq * 0.25).astype(BF)
        if nt == 1:
            og_v[...] = acc_g[...].T.astype(BF)
            ou_v[...] = acc_u[...].T.astype(BF)
            od_v[...] = acc_d[...].T.astype(BF)
            oo_v[...] = acc_o[...].astype(BF)

    with jax.named_scope("phD"):
        run_attn(attn_bwd)


    def phase_e(b, c):
        rows = pl.ds(pl.multiple_of(b * RB, RB), RB)
        cat = lambda ref: jnp.concatenate([ref[b * TPB + t] for t in range(TPB)], axis=1)
        dqkv = jnp.concatenate([cat(dqt), (cat(dkt) * (1.0 / LOG2E)).astype(BF), cat(dvt).astype(BF)], axis=0)
        dxn = _nn(wqkv_v[...], dqkv).T
        xn, r = _ln(x_v[rows, :].astype(F32))
        acc_qkv[...] += _nt(xn1t[b], dqkv)
        dx_v[rows, :] = (h_s[rows, :] + _ln_bwd(dxn, xn, r)).astype(BF)

        @pl.when(b == NRB - 2)
        def _():
            cp(dx_v.at[:S - 2 * RB], dx_hbm.at[:S - 2 * RB], 15).start()
        return c
    with jax.named_scope("phE"):
        lax.fori_loop(0, NRB, phase_e, 0)

    c1 = cp(dx_v.at[S - 2 * RB:], dx_hbm.at[S - 2 * RB:], 12)
    c1.start()
    oqkv_v[...] = acc_qkv[...].astype(BF)
    c2 = cp(oqkv_v, dwqkv_hbm, 13)
    c2.start()
    for c in out_cps + [c1, c2, cp(dx_v.at[:S - 2 * RB], dx_hbm.at[:S - 2 * RB], 15)]:
        c.wait()


@jax.jit
def pallas_sequential_preLN__sliding_block__glu_gated_glu__prompt_kernel(
    A_x: jax.Array,
    A_wqkv: jax.Array,
    A_wo: jax.Array,
    B_x: jax.Array,
    B_w_gate: jax.Array,
    B_w_up: jax.Array,
    B_w_down: jax.Array,
    grad_out: jax.Array,
):
    del B_x
    V = pltpu.VMEM
    tb = lambda dt: V((NT, D, T), dt)
    scratch = [
        V((S, D), BF), V((D, 3 * D), BF), V((D, D), BF), V((F, D), BF), V((F, D), BF), V((F, D), BF), V((S, D), BF),
        V((NRB, D, RB), BF), V((G, S, 128), BF), V((G, S, 128), BF), tb(BF), tb(BF), tb(BF), tb(BF),
        V((NT, G, 8, T), F32), V((NT, H, 2, T, T), BF), V((S, D), F32), tb(BF), V((NT, G, 8, T), F32),
        tb(BF), tb(F32), tb(F32),
        V((D, F), F32), V((D, F), F32), V((D, F), F32), V((D, D), F32), V((D, 3 * D), F32),
        V((S, D), BF), V((S, D), BF), V((F, D), BF), V((F, D), BF), V((F, D), BF), V((D, D), BF), V((D, 3 * D), BF),
        pltpu.SemaphoreType.DMA((16,)),
    ]
    sd = jax.ShapeDtypeStruct
    outs = pl.pallas_call(
        _kernel,
        out_shape=(sd((S, D), BF), sd((S, D), BF), sd((D, 3 * D), BF), sd((D, D), BF),
                   sd((F, D), BF), sd((F, D), BF), sd((F, D), BF)),
        in_specs=[pl.BlockSpec(memory_space=pl.ANY)] * 7,
        out_specs=[pl.BlockSpec(memory_space=pl.ANY)] * 7,
        scratch_shapes=scratch,
        compiler_params=pltpu.CompilerParams(vmem_limit_bytes=127 * 1024 * 1024),
    )(A_x.reshape(S, D), A_wqkv, A_wo, B_w_gate.T, B_w_up.T, B_w_down, grad_out.reshape(S, D))
    return (outs[0].reshape(1, S, D), outs[1].reshape(1, S, D)) + (outs[2], outs[3], outs[4].T, outs[5].T, outs[6])
```
